```python
import os as _os
_os.environ.setdefault('JAX_PLATFORMS', 'cpu')
import jax
import jax.numpy as jnp

def _softmax(x, axis=-1):
    return jax.nn.softmax(x, axis=axis)

def _gelu(x):
    return jax.nn.gelu(x, approximate=True)

def _silu(x):
    return jax.nn.silu(x)

def _sigmoid(x):
    return jax.nn.sigmoid(x)

def _layernorm(x, axis=-1, eps=1e-05):
    m = jnp.mean(x, axis=axis, keepdims=True)
    v = jnp.var(x, axis=axis, keepdims=True)
    return (x - m) / jnp.sqrt(v + eps)

def _scatter_add(tgt, idx, src, axis=0):
    return tgt.at[idx].add(src)

def _segment_sum(src, seg, n):
    return jax.ops.segment_sum(src, seg, n)

class _Rng:

    def __init__(self, key):
        self._k = key

    def _next(self):
        self._k, sub = jax.random.split(self._k)
        return sub

    def normal(self, shape):
        return jax.random.normal(self._next(), shape, dtype=jnp.bfloat16)

    def randint(self, lo, hi, shape):
        return jax.random.randint(self._next(), shape, lo, hi, dtype=jnp.int32)

    def uniform(self, shape, lo=0.0, hi=1.0):
        return jax.random.uniform(self._next(), shape, jnp.bfloat16, lo, hi)

    def permutation(self, n):
        return jax.random.permutation(self._next(), n)
kernel_name = 'adaLN_cond__mha_block__geglu_ffn__prompt'

def setup_inputs():
    _rng = _Rng(jax.random.key(int.from_bytes(__import__("os").urandom(4), "little")))
    _w = lambda a: (lambda t: t.astype(jnp.bfloat16) if jnp.issubdtype(t.dtype, jnp.floating) else t)(jnp.asarray(a))

    def _A_setup():
        B, S, D, H = (1, 2048, 640, 32)
        return {'x': _w((lambda *s: _rng.normal(s) * 0.05)(B, S, D)), 'wqkv': _w((lambda *s: _rng.normal(s) * 0.05)(D, 3 * D)), 'wo': _w((lambda *s: _rng.normal(s) * 0.05)(D, D))}
    _A_in = _A_setup()

    def _B_setup():
        B, S, D, F = (1, 2048, 640, 1728)
        return {'x': _w((lambda *s: _rng.normal(s) * 0.05)(B, S, D)), 'w_gate': _w((lambda *s: _rng.normal(s) * 0.05)(D, F)), 'w_up': _w((lambda *s: _rng.normal(s) * 0.05)(D, F)), 'w_down': _w((lambda *s: _rng.normal(s) * 0.05)(F, D))}
    _B_in = _B_setup()
    return {'A_x': _A_in['x'], 'A_wqkv': _A_in['wqkv'], 'A_wo': _A_in['wo'], 'B_x': _B_in['x'], 'B_w_gate': _B_in['w_gate'], 'B_w_up': _B_in['w_up'], 'B_w_down': _B_in['w_down'], 'c': _w((lambda *s: _rng.normal(s) * 0.05)(1, 640) * 8.0), 'w_mod': _w((lambda *s: _rng.normal(s) * 0.05)(640, 6 * 640) * 640 ** (-0.5) * 8.0)}

def reference(A_x, A_wqkv, A_wo, B_x, B_w_gate, B_w_up, B_w_down, c, w_mod):

    def _A_ref(x, wqkv, wo):
        B, S, D = x.shape
        H = 32
        Dh = D // H
        qkv = (lambda x, *d: x.transpose(*d))((x @ wqkv).reshape(B, S, 3, H, Dh), 2, 0, 3, 1, 4)
        q, k, v = (qkv[0], qkv[1], qkv[2])
        scores = jnp.einsum('bhqd,bhkd->bhqk', q, k) * Dh ** (-0.5)
        p = _softmax(scores, axis=-1)
        o = jnp.einsum('bhqk,bhkd->bhqd', p, v)
        return (lambda x, *d: x.transpose(*d))(o, 0, 2, 1, 3).reshape(B, S, D) @ wo

    def _B_ref(x, w_gate, w_up, w_down):
        return _gelu(x @ w_gate) * (x @ w_up) @ w_down
    x = A_x
    mod = (_silu(c) @ w_mod).reshape(c.shape[0], 6, 1, -1)
    sa, ca, ga, sb, cb, gb = (mod[:, 0].copy(), mod[:, 1].copy(), mod[:, 2].copy(), mod[:, 3].copy(), mod[:, 4].copy(), mod[:, 5].copy())
    h = _layernorm(x, axis=-1) * (1 + ca) + sa
    x = x + ga * _A_ref(h, A_wqkv, A_wo)
    h = _layernorm(x, axis=-1) * (1 + cb) + sb
    x = x + gb * _B_ref(h, B_w_gate, B_w_up, B_w_down)
    return x
```

```python
import jax
import jax.numpy as jnp
import jax.experimental.pallas as pl
import jax.experimental.pallas.tpu as pltpu

S = 2048
D = 640
H = 32
DH = 20
F = 1728
HPG = 6
G = 6
VR = 24
PADW = G * 128
TQ = 512
CK = 128
NQ = S // TQ
TB1 = 512
TB2 = 256
EPS = 1e-5
QSCALE = float(DH) ** -0.5 * 1.4426950408889634

F32 = jnp.float32
BF16 = jnp.bfloat16
NT = (((1,), (1,)), ((), ()))
TN = (((0,), (0,)), ((), ()))


def _ln_mod(xb, scale1p, shift):
    mu = jnp.mean(xb, axis=-1, keepdims=True)
    xc = xb - mu
    var = jnp.mean(xc * xc, axis=-1, keepdims=True)
    return xc * jax.lax.rsqrt(var + EPS) * scale1p + shift


def _pad_head_rows(w):
    z = jnp.zeros((VR - DH, w.shape[1]), F32)
    pieces = []
    for h in range(H):
        pieces.append(w[DH * h:DH * (h + 1), :])
        pieces.append(z)
    return jnp.concatenate(pieces, axis=0)


def _kernel(x_hbm, wqkv_hbm, wo_hbm, wg_hbm, wu_hbm, wd_hbm, c_hbm, wmod_hbm,
            out_hbm,
            x_s, wqkv_s, wo_s, wg_s, wu_s, wd_s, c_s, wmod_s,
            h_s, k_s, qt_s, vt_s, s_s, ot_s, wk_p, wqv_p, wo_p, mod_s, out_s,
            sems, out_sems):
    cp_c = pltpu.make_async_copy(c_hbm, c_s, sems.at[0])
    cp_wm0 = pltpu.make_async_copy(wmod_hbm.at[:, 0:2 * D], wmod_s.at[:, 0:2 * D], sems.at[1])
    cp_x = pltpu.make_async_copy(x_hbm, x_s, sems.at[2])
    cp_wqkv = pltpu.make_async_copy(wqkv_hbm, wqkv_s, sems.at[3])
    cp_wm1 = pltpu.make_async_copy(wmod_hbm.at[:, 2 * D:6 * D], wmod_s.at[:, 2 * D:6 * D], sems.at[4])
    cp_wo = pltpu.make_async_copy(wo_hbm, wo_s, sems.at[5])
    cp_wg = pltpu.make_async_copy(wg_hbm, wg_s, sems.at[6])
    cp_wu = pltpu.make_async_copy(wu_hbm, wu_s, sems.at[7])
    cp_wd = pltpu.make_async_copy(wd_hbm, wd_s, sems.at[8])
    cp_c.start()
    cp_wm0.start()
    cp_x.start()
    cp_wqkv.start()

    cp_c.wait()
    cf = c_s[...].astype(F32)
    sc = (cf * jax.nn.sigmoid(cf)).astype(BF16)
    sc8 = jnp.broadcast_to(sc, (8, D))
    cp_wm0.wait()
    mod_s[:, 0:2 * D] = jnp.dot(sc8, wmod_s[:, 0:2 * D], preferred_element_type=F32)

    cp_x.wait()

    def ln1_body(i, carry):
        rows = pl.ds(pl.multiple_of(i * TB2, TB2), TB2)
        sa = mod_s[0:1, 0:D]
        ca = mod_s[0:1, D:2 * D]
        h_s[rows, :] = _ln_mod(x_s[rows, :].astype(F32), 1.0 + ca, sa).astype(BF16)
        return carry

    jax.lax.fori_loop(0, S // TB2, ln1_body, 0)

    cp_wqkv.wait()
    cp_wm1.start()
    cp_wo.start()
    cp_wg.start()
    cp_wu.start()
    cp_wd.start()

    wk = wqkv_s[:, D:2 * D].astype(F32)
    pieces = []
    for g in range(G):
        n = min(HPG * DH, D - HPG * DH * g)
        pieces.append(wk[:, HPG * DH * g:HPG * DH * g + n])
        pieces.append(jnp.zeros((D, 128 - n), F32))
    wk_p[...] = jnp.concatenate(pieces, axis=1).astype(BF16)

    wqt = wqkv_s[:, 0:D].astype(F32).T
    pieces = []
    for g in range(G):
        n = min(HPG * DH, D - HPG * DH * g)
        pieces.append(wqt[HPG * DH * g:HPG * DH * g + n, :])
        pieces.append(jnp.zeros((128 - n, D), F32))
    wqv_p[0:PADW, :] = jnp.concatenate(pieces, axis=0).astype(BF16)
    wvt = wqkv_s[:, 2 * D:3 * D].astype(F32).T
    wqv_p[PADW:2 * PADW, :] = _pad_head_rows(wvt).astype(BF16)

    def qkv_body(i, carry):
        rows = pl.ds(pl.multiple_of(i * TB1, TB1), TB1)
        hb = h_s[rows, :]
        kb = jnp.dot(hb, wk_p[...], preferred_element_type=F32).astype(BF16)
        for g in range(G):
            k_s[g, rows, :] = kb[:, 128 * g:128 * (g + 1)]
        qv = jax.lax.dot_general(wqv_p[...], hb, NT, preferred_element_type=F32)
        for g in range(G):
            qt_s[g, :, rows] = (qv[128 * g:128 * (g + 1), :] * QSCALE).astype(BF16)
        r = jax.lax.broadcasted_iota(jnp.int32, (PADW, TB1), 0)
        vt_s[:, rows] = jnp.where(r % VR == DH, 1.0, qv[PADW:2 * PADW, :])
        return carry

    jax.lax.fori_loop(0, S // TB1, qkv_body, 0)

    def make_qm(it):
        h = it // NQ
        qt = it % NQ
        g = h // HPG
        off = (h % HPG) * DH
        row = jax.lax.broadcasted_iota(jnp.int32, (128, TQ), 0)
        qs = qt_s[g, :, pl.ds(pl.multiple_of(qt * TQ, TQ), TQ)]
        qm = jnp.where((row >= off) & (row < off + DH), qs, jnp.zeros_like(qs))
        return g, qm

    def pass1_chunk(g, qm, c, m8):
        s = jnp.dot(k_s[g, c * CK:(c + 1) * CK, :], qm, preferred_element_type=F32)
        s_s[c * CK:(c + 1) * CK, :] = s
        mc = jnp.max(s.reshape(CK // 8, 8, TQ), axis=0)
        return mc if m8 is None else jnp.maximum(m8, mc)

    def pass2_chunk(h, m, c, o):
        p = jnp.exp2(s_s[c * CK:(c + 1) * CK, :] - m)
        vrows = pl.ds(pl.multiple_of(h * VR, 8), VR)
        oc = jnp.dot(vt_s[vrows, c * CK:(c + 1) * CK], p, preferred_element_type=F32)
        return oc if o is None else o + oc

    def finish(it, o):
        h = it // NQ
        qt = it % NQ
        o = o / o[DH:DH + 1, :]
        ot_s[pl.ds(pl.multiple_of(h * VR, 8), VR), pl.ds(pl.multiple_of(qt * TQ, TQ), TQ)] = o

    g0, qm0 = make_qm(0)
    m8 = None
    for c in range(S // CK):
        m8 = pass1_chunk(g0, qm0, c, m8)
    m0 = jnp.max(m8, axis=0, keepdims=True)

    def attn_body(it, m):
        g, qm = make_qm(it)
        hp = (it - 1) // NQ
        m8 = None
        o = None
        for c in range(S // CK):
            o = pass2_chunk(hp, m, c, o)
            m8 = pass1_chunk(g, qm, c, m8)
        finish(it - 1, o)
        return jnp.max(m8, axis=0, keepdims=True)

    m = jax.lax.fori_loop(1, H * NQ, attn_body, m0)
    o = None
    for c in range(S // CK):
        o = pass2_chunk(H - 1, m, c, o)
    finish(H * NQ - 1, o)

    cp_wm1.wait()
    cf = c_s[...].astype(F32)
    sc8 = jnp.broadcast_to((cf * jax.nn.sigmoid(cf)).astype(BF16), (8, D))
    mod_s[:, 2 * D:6 * D] = jnp.dot(sc8, wmod_s[:, 2 * D:6 * D], preferred_element_type=F32)
    cp_wo.wait()
    wo_p[...] = _pad_head_rows(wo_s[...].astype(F32)).astype(BF16)
    cp_wg.wait()
    cp_wu.wait()
    cp_wd.wait()

    def out_copy(i, slot):
        rows = pl.ds(pl.multiple_of(i * TB2, TB2), TB2)
        return pltpu.make_async_copy(out_s.at[slot], out_hbm.at[rows, :], out_sems.at[slot])

    def ffn_body(i, carry):
        rows = pl.ds(pl.multiple_of(i * TB2, TB2), TB2)
        slot = i % 2
        ga = mod_s[0:1, 2 * D:3 * D]
        sb = mod_s[0:1, 3 * D:4 * D]
        cb = mod_s[0:1, 4 * D:5 * D]
        gb = mod_s[0:1, 5 * D:6 * D]
        attn = jax.lax.dot_general(ot_s[:, rows].astype(BF16), wo_p[...], TN,
                                   preferred_element_type=F32)
        x1 = x_s[rows, :].astype(F32) + ga * attn
        h2 = _ln_mod(x1, 1.0 + cb, sb).astype(BF16)
        gate = jax.lax.dot_general(h2, wg_s[...], NT, preferred_element_type=F32)
        up = jax.lax.dot_general(h2, wu_s[...], NT, preferred_element_type=F32)
        a = (jax.nn.gelu(gate, approximate=True) * up).astype(BF16)
        y = jnp.dot(a, wd_s[...], preferred_element_type=F32)

        @pl.when(i >= 2)
        def _():
            out_copy(i - 2, slot).wait()

        out_s[slot] = (x1 + gb * y).astype(BF16)
        out_copy(i, slot).start()
        return carry

    nblk = S // TB2
    jax.lax.fori_loop(0, nblk, ffn_body, 0)
    out_copy(nblk - 2, (nblk - 2) % 2).wait()
    out_copy(nblk - 1, (nblk - 1) % 2).wait()


@jax.jit
def pallas_adaLN_cond__mha_block__geglu_ffn__prompt_kernel(
    A_x: jax.Array,
    A_wqkv: jax.Array,
    A_wo: jax.Array,
    B_x: jax.Array,
    B_w_gate: jax.Array,
    B_w_up: jax.Array,
    B_w_down: jax.Array,
    c: jax.Array,
    w_mod: jax.Array,
):
    del B_x
    x = A_x.reshape(S, D)
    any_spec = pl.BlockSpec(memory_space=pltpu.MemorySpace.HBM)
    scratch = [
        pltpu.VMEM((S, D), BF16),
        pltpu.VMEM((D, 3 * D), BF16),
        pltpu.VMEM((D, D), BF16),
        pltpu.VMEM((F, D), BF16),
        pltpu.VMEM((F, D), BF16),
        pltpu.VMEM((F, D), BF16),
        pltpu.VMEM((1, D), BF16),
        pltpu.VMEM((D, 6 * D), BF16),
        pltpu.VMEM((S, D), BF16),
        pltpu.VMEM((G, S, 128), BF16),
        pltpu.VMEM((G, 128, S), BF16),
        pltpu.VMEM((PADW, S), F32),
        pltpu.VMEM((S, TQ), F32),
        pltpu.VMEM((PADW, S), F32),
        pltpu.VMEM((D, PADW), BF16),
        pltpu.VMEM((2 * PADW, D), BF16),
        pltpu.VMEM((PADW, D), BF16),
        pltpu.VMEM((8, 6 * D), F32),
        pltpu.VMEM((2, TB2, D), BF16),
        pltpu.SemaphoreType.DMA((9,)),
        pltpu.SemaphoreType.DMA((2,)),
    ]
    out = pl.pallas_call(
        _kernel,
        out_shape=jax.ShapeDtypeStruct((S, D), BF16),
        in_specs=[any_spec] * 8,
        out_specs=any_spec,
        scratch_shapes=scratch,
        compiler_params=pltpu.CompilerParams(vmem_limit_bytes=100 * 1024 * 1024),
    )(x, A_wqkv, A_wo, B_w_gate.T, B_w_up.T, B_w_down, c, w_mod)
    return out.reshape(1, S, D)
```

```python
import jax
import jax.numpy as jnp
import jax.experimental.pallas as pl
import jax.experimental.pallas.tpu as pltpu

S = 2048
D = 640
H = 32
DH = 20
F = 1728
HPG = 6
G = 6
VR = 24
PADW = G * 128
TQ = 512
CK = 128
NQ = S // TQ
NC = S // CK
UPB = 4
LAG = NC + 1
TB = 256
NBLK = S // TB
EPS = 1e-5
QSCALE = float(DH) ** -0.5 * 1.4426950408889634

F32 = jnp.float32
BF16 = jnp.bfloat16
NT = (((1,), (1,)), ((), ()))
TN = (((0,), (0,)), ((), ()))


def _ln_mod(xb, scale1p, shift):
    mu = jnp.mean(xb, axis=-1, keepdims=True)
    xc = xb - mu
    var = jnp.mean(xc * xc, axis=-1, keepdims=True)
    return xc * jax.lax.rsqrt(var + EPS) * scale1p + shift


def _pad_head_rows(w):
    z = jnp.zeros((VR - DH, w.shape[1]), F32)
    pieces = []
    for h in range(H):
        pieces.append(w[DH * h:DH * (h + 1), :])
        pieces.append(z)
    return jnp.concatenate(pieces, axis=0)


def _blk(i):
    if isinstance(i, int):
        return pl.ds(i * TB, TB)
    return pl.ds(pl.multiple_of(i * TB, TB), TB)


def _kernel(x_hbm, wqkv_hbm, wo_hbm, wgt_hbm, wut_hbm, wd_hbm, c_hbm, wmod_hbm,
            out_hbm,
            x_s, wqkv_s, wo_s, wgt_s, wut_s, wd_s, c_s, wmod_s,
            h_s, k_s, qt_s, vt_s, s0_s, s1_s, ot_s, wk_p, wqv_p, wo_p, mod_s,
            x1_s, h2_s, out_s,
            sems, x_sems, out_sems):
    cp_c = pltpu.make_async_copy(c_hbm, c_s, sems.at[0])
    cp_wm0 = pltpu.make_async_copy(wmod_hbm.at[:, 0:2 * D], wmod_s.at[:, 0:2 * D], sems.at[1])
    cp_wqkv = pltpu.make_async_copy(wqkv_hbm, wqkv_s, sems.at[3])
    cp_wm1 = pltpu.make_async_copy(wmod_hbm.at[:, 2 * D:6 * D], wmod_s.at[:, 2 * D:6 * D], sems.at[4])
    cp_wo = pltpu.make_async_copy(wo_hbm, wo_s, sems.at[5])
    cp_wg = pltpu.make_async_copy(wgt_hbm, wgt_s, sems.at[6])
    cp_wu = pltpu.make_async_copy(wut_hbm, wut_s, sems.at[7])
    cp_wd = pltpu.make_async_copy(wd_hbm, wd_s, sems.at[8])

    def cp_x(i):
        return pltpu.make_async_copy(x_hbm.at[_blk(i), :], x_s.at[_blk(i), :], x_sems.at[i])

    with jax.named_scope("p1_pro"):
        cp_wqkv.start()
        cp_c.start()
        cp_wm0.start()
        for i in range(NBLK):
            cp_x(i).start()

        cp_wqkv.wait()
        wk = wqkv_s[:, D:2 * D].astype(F32)
        pieces = []
        for g in range(G):
            n = min(HPG * DH, D - HPG * DH * g)
            pieces.append(wk[:, HPG * DH * g:HPG * DH * g + n])
            pieces.append(jnp.zeros((D, 128 - n), F32))
        wk_p[...] = jnp.concatenate(pieces, axis=1).astype(BF16)

        wqt = wqkv_s[:, 0:D].astype(F32).T
        pieces = []
        for g in range(G):
            n = min(HPG * DH, D - HPG * DH * g)
            pieces.append(wqt[HPG * DH * g:HPG * DH * g + n, :])
            pieces.append(jnp.zeros((128 - n, D), F32))
        wqv_p[0:PADW, :] = jnp.concatenate(pieces, axis=0).astype(BF16)
        wvt = wqkv_s[:, 2 * D:3 * D].astype(F32).T
        wqv_p[PADW:2 * PADW, :] = _pad_head_rows(wvt).astype(BF16)

        cp_c.wait()
        cf = c_s[...].astype(F32)
        sc8 = jnp.broadcast_to((cf * jax.nn.sigmoid(cf)).astype(BF16), (8, D))
        cp_wm0.wait()
        mod_s[:, 0:2 * D] = jnp.dot(sc8, wmod_s[:, 0:2 * D], preferred_element_type=F32)

        def ln1(i):
            sa = mod_s[0:1, 0:D]
            ca = mod_s[0:1, D:2 * D]
            h_s[_blk(i), :] = _ln_mod(x_s[_blk(i), :].astype(F32), 1.0 + ca, sa).astype(BF16)

        cp_x(0).wait()
        ln1(0)
        cp_wm1.start()
        cp_wo.start()
        cp_wg.start()
        cp_wu.start()
        cp_wd.start()

    def qkv_body(i, carry):
        nxt = jnp.minimum(i + 1, NBLK - 1)

        @pl.when(i + 1 < NBLK)
        def _():
            cp_x(nxt).wait()

        rows = _blk(i)
        hb = h_s[rows, :]
        kb = jnp.dot(hb, wk_p[...], preferred_element_type=F32).astype(BF16)
        for g in range(G):
            k_s[g, rows, :] = kb[:, 128 * g:128 * (g + 1)]
        ln1(nxt)
        qv = jax.lax.dot_general(wqv_p[...], hb, NT, preferred_element_type=F32)
        for g in range(G):
            qt_s[g, :, rows] = (qv[128 * g:128 * (g + 1), :] * QSCALE).astype(BF16)
        r = jax.lax.broadcasted_iota(jnp.int32, (PADW, TB), 0)
        vt_s[:, rows] = jnp.where(r % VR == DH, 1.0, qv[PADW:2 * PADW, :])
        return carry

    with jax.named_scope("p4_qkv"):
        jax.lax.fori_loop(0, NBLK, qkv_body, 0)

    s_refs = (s0_s, s1_s)

    def unit(hb, j):
        return hb + j // NQ, (j % NQ) * TQ

    def make_qm(h, col):
        g = h // HPG
        off = (h % HPG) * DH
        row = jax.lax.broadcasted_iota(jnp.int32, (128, TQ), 0)
        qs = qt_s[g, :, col:col + TQ]
        qm = jnp.where((row >= off) & (row < off + DH), qs, jnp.zeros_like(qs))
        return g, qm

    def s_rows(z, c):
        if isinstance(z, int):
            return pl.ds(z + c * CK, CK)
        return pl.ds(pl.multiple_of(z + c * CK, CK), CK)

    def qk(s_ref, g, qm, c, m8, z):
        s = jnp.dot(k_s[g, c * CK:(c + 1) * CK, :], qm, preferred_element_type=F32)
        s_ref[s_rows(z, c), :] = s
        mc = jnp.max(s.reshape(CK // 8, 8, TQ), axis=0)
        return mc if m8 is None else jnp.maximum(m8, mc)

    def pv(s_ref, h, m, c, o, z):
        p = jnp.exp2(s_ref[s_rows(z, c), :] - m)
        if isinstance(h, int):
            vrows = pl.ds(h * VR, VR)
        else:
            vrows = pl.ds(pl.multiple_of(h * VR, 8), VR)
        oc = jnp.dot(vt_s[vrows, c * CK:(c + 1) * CK], p, preferred_element_type=F32)
        return oc if o is None else o + oc

    def finish(h, col, o):
        o = o / o[DH:DH + 1, :]
        if isinstance(h, int):
            vrows = pl.ds(h * VR, VR)
        else:
            vrows = pl.ds(pl.multiple_of(h * VR, 8), VR)
        ot_s[vrows, col:col + TQ] = o

    def attn_body(hb, carry, last=False):
        if isinstance(hb, int):
            z1 = z2 = 0
        else:
            z1 = jax.lax.shift_right_logical(hb, 16) * CK
            z2 = jax.lax.shift_right_logical(hb, 17) * CK
        m8d = {0: carry[0], 1: carry[1]}
        qms = {}
        o = None
        m = None
        for t in range(UPB * NC):
            j, c = divmod(t, NC)
            if c == 0:
                m = jnp.max(m8d[j], axis=0, keepdims=True)
                o = None
            h, col = unit(hb, j)
            o = pv(s_refs[j % 2], h, m, c, o, z2)
            if c == NC - 1:
                finish(h, col, o)
            jq, cq = divmod(t + LAG, NC)
            if last and jq >= UPB:
                continue
            if jq not in qms:
                qms[jq] = make_qm(*unit(hb, jq))
            g, qm = qms[jq]
            m8d[jq] = qk(s_refs[jq % 2], g, qm, cq, m8d.get(jq), z1)
        if last:
            return None
        return (m8d[UPB], m8d[UPB + 1])

    with jax.named_scope("p5_attn"):
        m8s = {}
        m8 = None
        for t in range(LAG):
            j, c = divmod(t, NC)
            if c == 0:
                g, qm = make_qm(*unit(0, j))
                m8 = None
            m8 = qk(s_refs[j % 2], g, qm, c, m8, 0)
            m8s[j] = m8
        carry = jax.lax.fori_loop(0, H - 1, attn_body, (m8s[0], m8s[1]))
        attn_body(H - 1, carry, last=True)

    with jax.named_scope("p6_mod2"):
        cp_wm1.wait()
        cf = c_s[...].astype(F32)
        sc8 = jnp.broadcast_to((cf * jax.nn.sigmoid(cf)).astype(BF16), (8, D))
        mod_s[:, 2 * D:6 * D] = jnp.dot(sc8, wmod_s[:, 2 * D:6 * D], preferred_element_type=F32)
        cp_wo.wait()
        wo_p[...] = _pad_head_rows(wo_s[...].astype(F32)).astype(BF16)
        cp_wg.wait()
        cp_wu.wait()
        cp_wd.wait()

    def out_copy(i, slot):
        return pltpu.make_async_copy(out_s.at[slot], out_hbm.at[_blk(i), :], out_sems.at[slot])

    def stage_a1(i):
        return jax.lax.dot_general(ot_s[:, _blk(i)].astype(BF16), wo_p[...], TN,
                                   preferred_element_type=F32)

    def stage_a2(i, attn):
        ga = mod_s[0:1, 2 * D:3 * D]
        sb = mod_s[0:1, 3 * D:4 * D]
        cb = mod_s[0:1, 4 * D:5 * D]
        x1 = x_s[_blk(i), :].astype(F32) + ga * attn
        x1_s[i % 2] = x1
        h2_s[i % 2] = _ln_mod(x1, 1.0 + cb, sb).astype(BF16)

    def ffn_body(i, carry, last=False):
        slot = i % 2
        gb = mod_s[0:1, 5 * D:6 * D]
        h2 = h2_s[slot]
        gate = jax.lax.dot_general(h2, wgt_s[...], NT, preferred_element_type=F32)
        if not last:
            attn = stage_a1(i + 1)
        up = jax.lax.dot_general(h2, wut_s[...], NT, preferred_element_type=F32)
        if not last:
            stage_a2(i + 1, attn)
        a = (jax.nn.gelu(gate, approximate=True) * up).astype(BF16)
        y = jnp.dot(a, wd_s[...], preferred_element_type=F32)
        res = (x1_s[slot] + gb * y).astype(BF16)

        if last:
            out_copy(i - 2, slot).wait()
        else:
            @pl.when(i >= 2)
            def _():
                out_copy(i - 2, slot).wait()

        out_s[slot] = res
        out_copy(i, slot).start()
        return carry

    with jax.named_scope("p7_ffn"):
        stage_a2(0, stage_a1(0))
        jax.lax.fori_loop(0, NBLK - 1, ffn_body, 0)
        ffn_body(NBLK - 1, 0, last=True)
        out_copy(NBLK - 2, (NBLK - 2) % 2).wait()
        out_copy(NBLK - 1, (NBLK - 1) % 2).wait()


@jax.jit
def pallas_adaLN_cond__mha_block__geglu_ffn__prompt_kernel(
    A_x: jax.Array,
    A_wqkv: jax.Array,
    A_wo: jax.Array,
    B_x: jax.Array,
    B_w_gate: jax.Array,
    B_w_up: jax.Array,
    B_w_down: jax.Array,
    c: jax.Array,
    w_mod: jax.Array,
):
    del B_x
    x = A_x.reshape(S, D)
    hbm = pl.BlockSpec(memory_space=pltpu.MemorySpace.HBM)
    scratch = [
        pltpu.VMEM((S, D), BF16),
        pltpu.VMEM((D, 3 * D), BF16),
        pltpu.VMEM((D, D), BF16),
        pltpu.VMEM((F, D), BF16),
        pltpu.VMEM((F, D), BF16),
        pltpu.VMEM((F, D), BF16),
        pltpu.VMEM((1, D), BF16),
        pltpu.VMEM((D, 6 * D), BF16),
        pltpu.VMEM((S, D), BF16),
        pltpu.VMEM((G, S, 128), BF16),
        pltpu.VMEM((G, 128, S), BF16),
        pltpu.VMEM((PADW, S), F32),
        pltpu.VMEM((S, TQ), F32),
        pltpu.VMEM((S, TQ), F32),
        pltpu.VMEM((PADW, S), F32),
        pltpu.VMEM((D, PADW), BF16),
        pltpu.VMEM((2 * PADW, D), BF16),
        pltpu.VMEM((PADW, D), BF16),
        pltpu.VMEM((8, 6 * D), F32),
        pltpu.VMEM((2, TB, D), F32),
        pltpu.VMEM((2, TB, D), BF16),
        pltpu.VMEM((2, TB, D), BF16),
        pltpu.SemaphoreType.DMA((9,)),
        pltpu.SemaphoreType.DMA((NBLK,)),
        pltpu.SemaphoreType.DMA((2,)),
    ]
    out = pl.pallas_call(
        _kernel,
        out_shape=jax.ShapeDtypeStruct((S, D), BF16),
        in_specs=[hbm] * 8,
        out_specs=hbm,
        scratch_shapes=scratch,
        compiler_params=pltpu.CompilerParams(vmem_limit_bytes=100 * 1024 * 1024),
    )(x, A_wqkv, A_wo, B_w_gate.T, B_w_up.T, B_w_down, c, w_mod)
    return out.reshape(1, S, D)
```

```python
import jax
import jax.numpy as jnp
import jax.experimental.pallas as pl
import jax.experimental.pallas.tpu as pltpu

S = 2048
D = 640
H = 32
DH = 20
F = 1728
FM = 1664
FR = F - FM
HPG = 6
G = 6
GW = HPG * DH
VR = 24
PADW = G * 128
TQ = 512
CK = 128
NQ = S // TQ
NC = S // CK
UPB = 4
DEP_LAG = 2
DEP_ROW = 2
LAG = NC + 1
TB = 256
NBLK = S // TB
EPS = 1e-5
FCH = [(0, 512), (512, 896), (896, 1280), (1280, 1664), (1664, 1728)]
A1_AT = 0
A2_AT = 2
QSCALE = float(DH) ** -0.5 * 1.4426950408889634

F32 = jnp.float32
BF16 = jnp.bfloat16
NT = (((1,), (1,)), ((), ()))
TN = (((0,), (0,)), ((), ()))


def _ln_mod(xb, scale1p, shift):
    mu = jnp.mean(xb, axis=-1, keepdims=True)
    xc = xb - mu
    var = jnp.mean(xc * xc, axis=-1, keepdims=True)
    return xc * jax.lax.rsqrt(var + EPS) * scale1p + shift


def _pad_head_rows(w):
    z = jnp.zeros((VR - DH, w.shape[1]), F32)
    pieces = []
    for h in range(H):
        pieces.append(w[DH * h:DH * (h + 1), :])
        pieces.append(z)
    return jnp.concatenate(pieces, axis=0)


def _blk(i):
    if isinstance(i, int):
        return pl.ds(i * TB, TB)
    return pl.ds(pl.multiple_of(i * TB, TB), TB)


def _kernel(x_hbm, wqkv_hbm, wo_hbm, wgt_hbm, wut_hbm, wd_hbm, c_hbm, wmod_hbm,
            out_hbm,
            x_s, wqkv_s, wo_s, wgt_s, wut_s, wd_s, c_s, wmod_s,
            h_s, k_s, qt_s, vt_s, s0_s, s1_s, ot_s, wqv_p, wr_s, wdr_s, mod_s,
            x1_s, h2_s, out_s,
            sems, x_sems, out_sems):
    cp_c = pltpu.make_async_copy(c_hbm, c_s, sems.at[0])
    cp_wm0 = pltpu.make_async_copy(wmod_hbm.at[:, 0:2 * D], wmod_s.at[:, 0:2 * D], sems.at[1])
    cp_wqkv = pltpu.make_async_copy(wqkv_hbm, wqkv_s, sems.at[3])
    cp_wm1 = pltpu.make_async_copy(wmod_hbm.at[:, 2 * D:6 * D], wmod_s.at[:, 2 * D:6 * D], sems.at[4])
    cp_wo = pltpu.make_async_copy(wo_hbm, wo_s, sems.at[5])
    cp_wg = pltpu.make_async_copy(wgt_hbm, wgt_s, sems.at[6])
    cp_wu = pltpu.make_async_copy(wut_hbm, wut_s, sems.at[7])
    cp_wd = pltpu.make_async_copy(wd_hbm, wd_s, sems.at[8])

    def cp_x(i):
        return pltpu.make_async_copy(x_hbm.at[_blk(i), :], x_s.at[_blk(i), :], x_sems.at[i])

    with jax.named_scope("p1_pro"):
        cp_wqkv.start()
        cp_c.start()
        cp_wm0.start()
        cp_x(0).start()

        cp_wqkv.wait()
        for i in range(1, NBLK):
            cp_x(i).start()
        wqv_p[0:D, :] = wqkv_s[:, 0:D].astype(F32).T.astype(BF16)
        wqv_p[D:2 * D, :] = wqkv_s[:, 2 * D:3 * D].astype(F32).T.astype(BF16)

        cp_c.wait()
        cf = c_s[...].astype(F32)
        sc8 = jnp.broadcast_to((cf * jax.nn.sigmoid(cf)).astype(BF16), (8, D))
        cp_wm0.wait()
        mod_s[:, 0:2 * D] = jnp.dot(sc8, wmod_s[:, 0:2 * D], preferred_element_type=F32)

        def ln1(i):
            sa = mod_s[0:1, 0:D]
            ca = mod_s[0:1, D:2 * D]
            h_s[_blk(i), :] = _ln_mod(x_s[_blk(i), :].astype(F32), 1.0 + ca, sa).astype(BF16)

        cp_x(0).wait()
        ln1(0)
        cp_wm1.start()
        cp_wo.start()
        cp_wg.start()
        cp_wu.start()
        cp_wd.start()

    def qkv_body(i, carry):
        nxt = jnp.minimum(i + 1, NBLK - 1)

        @pl.when(i + 1 < NBLK)
        def _():
            cp_x(nxt).wait()

        rows = _blk(i)
        hb = h_s[rows, :]
        kb = jnp.dot(hb, wqkv_s[:, D:2 * D], preferred_element_type=F32)
        for g in range(G):
            n = min(GW, D - GW * g)
            kg = kb[:, GW * g:GW * g + n]
            kg = jnp.concatenate([kg, jnp.zeros((TB, 128 - n), F32)], axis=1)
            k_s[g, rows, :] = kg.astype(BF16)
        qq = jax.lax.dot_general(wqv_p[0:D, :], hb, NT, preferred_element_type=F32)
        for g in range(G):
            n = min(GW, D - GW * g)
            qt_s[g, 0:n, rows] = (qq[GW * g:GW * g + n, :] * QSCALE).astype(BF16)
        ln1(nxt)
        vv = jax.lax.dot_general(wqv_p[D:2 * D, :], hb, NT, preferred_element_type=F32)
        r = jax.lax.broadcasted_iota(jnp.int32, (PADW, TB), 0)
        vt_s[:, rows] = jnp.where(r % VR == DH, 1.0, _pad_head_rows(vv))
        return carry

    with jax.named_scope("p4_qkv"):
        jax.lax.fori_loop(0, NBLK, qkv_body, 0)

    def stage_a1(i):
        ot = ot_s[:, _blk(i)]
        oc = jnp.concatenate([ot[VR * h:VR * h + DH, :] for h in range(H)], axis=0)
        return jax.lax.dot_general(oc.astype(BF16), wo_s[...], TN, preferred_element_type=F32)

    def stage_a2(i, attn):
        ga = mod_s[0:1, 2 * D:3 * D]
        sb = mod_s[0:1, 3 * D:4 * D]
        cb = mod_s[0:1, 4 * D:5 * D]
        x1 = x_s[_blk(i), :].astype(F32) + ga * attn
        x1_s[i % 2] = x1
        h2_s[i % 2] = _ln_mod(x1, 1.0 + cb, sb).astype(BF16)

    s_refs = (s0_s, s1_s)
    deps = []

    def unit(hb, j):
        return hb + j // NQ, (j % NQ) * TQ

    def make_qm(h, col):
        g = h // HPG
        off = (h % HPG) * DH
        row = jax.lax.broadcasted_iota(jnp.int32, (128, TQ), 0)
        qs = qt_s[g, :, col:col + TQ]
        qm = jnp.where((row >= off) & (row < off + DH), qs, jnp.zeros_like(qs))
        return g, qm

    def s_rows(z, c):
        if isinstance(z, int):
            return pl.ds(z + c * CK, CK)
        return pl.ds(pl.multiple_of(z + c * CK, CK), CK)

    def qk(s_ref, g, qm, c, m8, z):
        s = jnp.dot(k_s[g, c * CK:(c + 1) * CK, :], qm, preferred_element_type=F32)
        s_ref[s_rows(z, c), :] = s
        mc = jnp.max(s.reshape(CK // 8, 8, TQ), axis=0)
        deps.append(s[DEP_ROW * 8:DEP_ROW * 8 + 8, :])
        return mc if m8 is None else jnp.maximum(m8, mc)

    def pv(s_ref, h, m, c, o, z, zv=None):
        sv = s_ref[s_rows(z, c), :]
        if zv is not None and len(deps) >= DEP_LAG:
            d = jax.lax.bitcast_convert_type(deps[-DEP_LAG], jnp.int32) & zv
            mb = jax.lax.bitcast_convert_type(jnp.broadcast_to(m, (8, TQ)), jnp.int32) | d
            mb = jax.lax.bitcast_convert_type(mb, F32)
            p = jnp.exp2(sv.reshape(CK // 8, 8, TQ) - mb[None]).reshape(CK, TQ)
        else:
            p = jnp.exp2(sv - m)
        if isinstance(h, int):
            vrows = pl.ds(h * VR, VR)
        else:
            vrows = pl.ds(pl.multiple_of(h * VR, 8), VR)
        oc = jnp.dot(vt_s[vrows, c * CK:(c + 1) * CK], p, preferred_element_type=F32)
        return oc if o is None else o + oc

    def finish(h, col, o):
        o = o / o[DH:DH + 1, :]
        if isinstance(h, int):
            vrows = pl.ds(h * VR, VR)
        else:
            vrows = pl.ds(pl.multiple_of(h * VR, 8), VR)
        ot_s[vrows, col:col + TQ] = o

    def attn_body(hb, carry, last=False):
        if isinstance(hb, int):
            z1 = z2 = 0
        else:
            z1 = jax.lax.shift_right_logical(hb, 16) * CK
            z2 = jax.lax.shift_right_logical(hb, 17) * CK
        deps.clear()
        zv = None if isinstance(hb, int) else jnp.broadcast_to(z1, (8, TQ))
        m8d = {0: carry[0], 1: carry[1]}
        qms = {}
        o = None
        m = None
        for t in range(UPB * NC):
            j, c = divmod(t, NC)
            if c == 0:
                m = jnp.max(m8d[j], axis=0, keepdims=True)
                o = None
            h, col = unit(hb, j)
            o = pv(s_refs[j % 2], h, m, c, o, z2, zv)
            if c == NC - 1:
                finish(h, col, o)
            jq, cq = divmod(t + LAG, NC)
            if last and jq >= UPB:
                if t + LAG == UPB * NC:
                    stage_a2(0, stage_a1(0))
                continue
            if jq not in qms:
                qms[jq] = make_qm(*unit(hb, jq))
            g, qm = qms[jq]
            m8d[jq] = qk(s_refs[jq % 2], g, qm, cq, m8d.get(jq), z1)
        if last:
            return None
        return (m8d[UPB], m8d[UPB + 1])

    with jax.named_scope("p5_attn"):
        cp_wm1.wait()
        cf = c_s[...].astype(F32)
        sc8 = jnp.broadcast_to((cf * jax.nn.sigmoid(cf)).astype(BF16), (8, D))
        mod_s[:, 2 * D:6 * D] = jnp.dot(sc8, wmod_s[:, 2 * D:6 * D], preferred_element_type=F32)
        cp_wo.wait()
        cp_wg.wait()
        cp_wu.wait()
        cp_wd.wait()
        wr_s[0:FR, :] = wgt_s[FM:F, :]
        wr_s[FR:2 * FR, :] = wut_s[FM:F, :]
        wdr_s[0:FR, :] = wd_s[FM:F, :]
        wdr_s[FR:2 * FR, :] = jnp.zeros((FR, D), BF16)
        m8s = {}
        m8 = None
        for t in range(LAG):
            j, c = divmod(t, NC)
            if c == 0:
                g, qm = make_qm(*unit(0, j))
                m8 = None
            m8 = qk(s_refs[j % 2], g, qm, c, m8, 0)
            m8s[j] = m8
        carry = jax.lax.fori_loop(0, H - 1, attn_body, (m8s[0], m8s[1]))
        attn_body(H - 1, carry, last=True)

    def out_copy(i, slot):
        return pltpu.make_async_copy(out_s.at[slot], out_hbm.at[_blk(i), :], out_sems.at[slot])

    def ffn_body(i, carry, last=False):
        slot = i % 2
        gb = mod_s[0:1, 5 * D:6 * D]

        def gu(lo, hi):
            h2 = h2_s[slot]
            gate = jax.lax.dot_general(h2, wgt_s[lo:hi, :], NT, preferred_element_type=F32)
            up = jax.lax.dot_general(h2, wut_s[lo:hi, :], NT, preferred_element_type=F32)
            return (jax.nn.gelu(gate, approximate=True) * up).astype(BF16)

        def gu_rem():
            h2 = h2_s[slot]
            rem = jax.lax.dot_general(h2, wr_s[...], NT, preferred_element_type=F32)
            return (jax.nn.gelu(rem, approximate=True) * pltpu.roll(rem, FR, axis=1)).astype(BF16)

        y = None
        prev = None
        for ci in range(len(FCH) + 1):
            cur = None
            if ci < len(FCH):
                lo, hi = FCH[ci]
                cur = (gu(lo, hi), wd_s, lo, hi) if hi <= FM else (gu_rem(), wdr_s, 0, 2 * FR)
            if ci == A1_AT and not last:
                attn = stage_a1(i + 1)
            if ci == A2_AT and not last:
                stage_a2(i + 1, attn)
            if prev is not None:
                a, w_ref, lo, hi = prev
                yc = jnp.dot(a, w_ref[lo:hi, :], preferred_element_type=F32)
                y = yc if y is None else y + yc
            prev = cur
        res = (x1_s[slot] + gb * y).astype(BF16)

        if last:
            out_copy(i - 2, slot).wait()
        else:
            @pl.when(i >= 2)
            def _():
                out_copy(i - 2, slot).wait()

        out_s[slot] = res
        out_copy(i, slot).start()
        return carry

    with jax.named_scope("p7_ffn"):
        jax.lax.fori_loop(0, NBLK - 1, ffn_body, 0)
        ffn_body(NBLK - 1, 0, last=True)
        out_copy(NBLK - 2, (NBLK - 2) % 2).wait()
        out_copy(NBLK - 1, (NBLK - 1) % 2).wait()


@jax.jit
def pallas_adaLN_cond__mha_block__geglu_ffn__prompt_kernel(
    A_x: jax.Array,
    A_wqkv: jax.Array,
    A_wo: jax.Array,
    B_x: jax.Array,
    B_w_gate: jax.Array,
    B_w_up: jax.Array,
    B_w_down: jax.Array,
    c: jax.Array,
    w_mod: jax.Array,
):
    del B_x
    x = A_x.reshape(S, D)
    hbm = pl.BlockSpec(memory_space=pltpu.MemorySpace.HBM)
    scratch = [
        pltpu.VMEM((S, D), BF16),
        pltpu.VMEM((D, 3 * D), BF16),
        pltpu.VMEM((D, D), BF16),
        pltpu.VMEM((F, D), BF16),
        pltpu.VMEM((F, D), BF16),
        pltpu.VMEM((F, D), BF16),
        pltpu.VMEM((1, D), BF16),
        pltpu.VMEM((D, 6 * D), BF16),
        pltpu.VMEM((S, D), BF16),
        pltpu.VMEM((G, S, 128), BF16),
        pltpu.VMEM((G, 128, S), BF16),
        pltpu.VMEM((PADW, S), F32),
        pltpu.VMEM((S, TQ), F32),
        pltpu.VMEM((S, TQ), F32),
        pltpu.VMEM((PADW, S), F32),
        pltpu.VMEM((2 * D, D), BF16),
        pltpu.VMEM((2 * FR, D), BF16),
        pltpu.VMEM((2 * FR, D), BF16),
        pltpu.VMEM((8, 6 * D), F32),
        pltpu.VMEM((2, TB, D), F32),
        pltpu.VMEM((2, TB, D), BF16),
        pltpu.VMEM((2, TB, D), BF16),
        pltpu.SemaphoreType.DMA((9,)),
        pltpu.SemaphoreType.DMA((NBLK,)),
        pltpu.SemaphoreType.DMA((2,)),
    ]
    out = pl.pallas_call(
        _kernel,
        out_shape=jax.ShapeDtypeStruct((S, D), BF16),
        in_specs=[hbm] * 8,
        out_specs=hbm,
        scratch_shapes=scratch,
        compiler_params=pltpu.CompilerParams(vmem_limit_bytes=100 * 1024 * 1024),
    )(x, A_wqkv, A_wo, B_w_gate.T, B_w_up.T, B_w_down, c, w_mod)
    return out.reshape(1, S, D)
```

```python
import jax
import jax.numpy as jnp
import jax.experimental.pallas as pl
import jax.experimental.pallas.tpu as pltpu

S = 2048
D = 640
H = 32
DH = 20
F = 1728
FM = 1664
FR = F - FM
HPG = 6
G = 6
GW = HPG * DH
VR = 24
PADW = G * 128
TQ = 512
CK = 128
NQ = S // TQ
NC = S // CK
UPB = 4
DEP_LAG = 2
DEP_ROW = 2
LAG = NC + 1
TB = 256
NBLK = S // TB
EPS = 1e-5
FCH = [(0, 512), (512, 896), (896, 1280), (1280, 1664), (1664, 1728)]
A1_AT = 0
A2_AT = 2
QSCALE = float(DH) ** -0.5 * 1.4426950408889634

F32 = jnp.float32
BF16 = jnp.bfloat16
NT = (((1,), (1,)), ((), ()))
TN = (((0,), (0,)), ((), ()))


def _ln_mod(xb, scale1p, shift):
    mu = jnp.mean(xb, axis=-1, keepdims=True)
    xc = xb - mu
    var = jnp.mean(xc * xc, axis=-1, keepdims=True)
    return xc * jax.lax.rsqrt(var + EPS) * scale1p + shift


def _pad_head_rows(w):
    z = jnp.zeros((VR - DH, w.shape[1]), F32)
    pieces = []
    for h in range(H):
        pieces.append(w[DH * h:DH * (h + 1), :])
        pieces.append(z)
    return jnp.concatenate(pieces, axis=0)


def _blk(i):
    if isinstance(i, int):
        return pl.ds(i * TB, TB)
    return pl.ds(pl.multiple_of(i * TB, TB), TB)


def _kernel(x_hbm, wqkv_hbm, wo_hbm, wgt_hbm, wut_hbm, wd_hbm, c_hbm, wmod_hbm,
            out_hbm,
            x_s, wqkv_s, wo_s, wgt_s, wut_s, wd_s, c_s, wmod_s,
            h_s, k_s, qt_s, vt_s, s0_s, s1_s, ot_s, wqv_p, wr_s, wdr_s, mod_s,
            x1_s, h2_s, out_s,
            sems, x_sems, out_sems):
    cp_c = pltpu.make_async_copy(c_hbm, c_s, sems.at[0])
    cp_wm0 = pltpu.make_async_copy(wmod_hbm.at[:, 0:2 * D], wmod_s.at[:, 0:2 * D], sems.at[1])
    cp_wq = pltpu.make_async_copy(wqkv_hbm.at[:, 0:D], wqkv_s.at[:, 0:D], sems.at[2])
    cp_wk = pltpu.make_async_copy(wqkv_hbm.at[:, D:2 * D], wqkv_s.at[:, D:2 * D], sems.at[3])
    cp_wv = pltpu.make_async_copy(wqkv_hbm.at[:, 2 * D:3 * D], wqkv_s.at[:, 2 * D:3 * D], sems.at[9])
    cp_wm1 = pltpu.make_async_copy(wmod_hbm.at[:, 2 * D:6 * D], wmod_s.at[:, 2 * D:6 * D], sems.at[4])
    cp_wo = pltpu.make_async_copy(wo_hbm, wo_s, sems.at[5])
    cp_wg = pltpu.make_async_copy(wgt_hbm, wgt_s, sems.at[6])
    cp_wu = pltpu.make_async_copy(wut_hbm, wut_s, sems.at[7])
    cp_wd = pltpu.make_async_copy(wd_hbm, wd_s, sems.at[8])

    def cp_x(i):
        return pltpu.make_async_copy(x_hbm.at[_blk(i), :], x_s.at[_blk(i), :], x_sems.at[i])

    def ln1(i):
        sa = mod_s[0:1, 0:D]
        ca = mod_s[0:1, D:2 * D]
        h_s[_blk(i), :] = _ln_mod(x_s[_blk(i), :].astype(F32), 1.0 + ca, sa).astype(BF16)

    def k_proj(i):
        rows = _blk(i)
        kb = jnp.dot(h_s[rows, :], wqkv_s[:, D:2 * D], preferred_element_type=F32)
        for g in range(G):
            n = min(GW, D - GW * g)
            kg = kb[:, GW * g:GW * g + n]
            kg = jnp.concatenate([kg, jnp.zeros((TB, 128 - n), F32)], axis=1)
            k_s[g, rows, :] = kg.astype(BF16)

    def q_proj(i):
        rows = _blk(i)
        qq = jax.lax.dot_general(wqv_p[0:D, :], h_s[rows, :], NT, preferred_element_type=F32)
        for g in range(G):
            n = min(GW, D - GW * g)
            qt_s[g, 0:n, rows] = (qq[GW * g:GW * g + n, :] * QSCALE).astype(BF16)

    def v_proj(i):
        rows = _blk(i)
        vv = jax.lax.dot_general(wqv_p[D:2 * D, :], h_s[rows, :], NT, preferred_element_type=F32)
        r = jax.lax.broadcasted_iota(jnp.int32, (PADW, TB), 0)
        vt_s[:, rows] = jnp.where(r % VR == DH, 1.0, _pad_head_rows(vv))

    cp_c.start()
    cp_wm0.start()
    cp_x(0).start()
    cp_wk.start()
    cp_c.wait()
    cf = c_s[...].astype(F32)
    sc8 = jnp.broadcast_to((cf * jax.nn.sigmoid(cf)).astype(BF16), (8, D))
    cp_wm0.wait()
    cp_wq.start()
    cp_x(1).start()
    mod_s[:, 0:2 * D] = jnp.dot(sc8, wmod_s[:, 0:2 * D], preferred_element_type=F32)
    cp_x(0).wait()
    ln1(0)
    cp_wk.wait()
    cp_wv.start()
    k_proj(0)
    cp_wq.wait()
    for i in range(2, NBLK):
        cp_x(i).start()
    wqv_p[0:D, :] = wqkv_s[:, 0:D].astype(F32).T.astype(BF16)
    q_proj(0)
    cp_x(1).wait()
    ln1(1)
    cp_wv.wait()
    cp_wm1.start()
    cp_wo.start()
    cp_wg.start()
    cp_wu.start()
    cp_wd.start()
    wqv_p[D:2 * D, :] = wqkv_s[:, 2 * D:3 * D].astype(F32).T.astype(BF16)
    v_proj(0)

    def qkv_body(i, carry):
        nxt = jnp.minimum(i + 1, NBLK - 1)

        @pl.when(i + 1 < NBLK)
        def _():
            cp_x(nxt).wait()

        k_proj(i)
        q_proj(i)
        ln1(nxt)
        v_proj(i)
        return carry

    jax.lax.fori_loop(1, NBLK, qkv_body, 0)

    def stage_a1(i):
        ot = ot_s[:, _blk(i)]
        oc = jnp.concatenate([ot[VR * h:VR * h + DH, :] for h in range(H)], axis=0)
        return jax.lax.dot_general(oc.astype(BF16), wo_s[...], TN, preferred_element_type=F32)

    def stage_a2(i, attn):
        ga = mod_s[0:1, 2 * D:3 * D]
        sb = mod_s[0:1, 3 * D:4 * D]
        cb = mod_s[0:1, 4 * D:5 * D]
        x1 = x_s[_blk(i), :].astype(F32) + ga * attn
        x1_s[i % 2] = x1
        h2_s[i % 2] = _ln_mod(x1, 1.0 + cb, sb).astype(BF16)

    s_refs = (s0_s, s1_s)
    deps = []

    def unit(hb, j):
        return hb + j // NQ, (j % NQ) * TQ

    def make_qm(h, col):
        g = h // HPG
        off = (h % HPG) * DH
        row = jax.lax.broadcasted_iota(jnp.int32, (128, TQ), 0)
        qs = qt_s[g, :, col:col + TQ]
        qm = jnp.where((row >= off) & (row < off + DH), qs, jnp.zeros_like(qs))
        return g, qm

    def s_rows(z, c):
        if isinstance(z, int):
            return pl.ds(z + c * CK, CK)
        return pl.ds(pl.multiple_of(z + c * CK, CK), CK)

    def qk(s_ref, g, qm, c, m8, z):
        s = jnp.dot(k_s[g, c * CK:(c + 1) * CK, :], qm, preferred_element_type=F32)
        s_ref[s_rows(z, c), :] = s
        mc = jnp.max(s.reshape(CK // 8, 8, TQ), axis=0)
        deps.append(s[DEP_ROW * 8:DEP_ROW * 8 + 8, :])
        return mc if m8 is None else jnp.maximum(m8, mc)

    def pv(s_ref, h, m, c, o, z, zv=None):
        sv = s_ref[s_rows(z, c), :]
        if zv is not None and len(deps) >= DEP_LAG:
            d = jax.lax.bitcast_convert_type(deps[-DEP_LAG], jnp.int32) & zv
            mb = jax.lax.bitcast_convert_type(jnp.broadcast_to(m, (8, TQ)), jnp.int32) | d
            mb = jax.lax.bitcast_convert_type(mb, F32)
            p = jnp.exp2(sv.reshape(CK // 8, 8, TQ) - mb[None]).reshape(CK, TQ)
        else:
            p = jnp.exp2(sv - m)
        if isinstance(h, int):
            vrows = pl.ds(h * VR, VR)
        else:
            vrows = pl.ds(pl.multiple_of(h * VR, 8), VR)
        oc = jnp.dot(vt_s[vrows, c * CK:(c + 1) * CK], p, preferred_element_type=F32)
        return oc if o is None else o + oc

    def finish(h, col, o):
        o = o / o[DH:DH + 1, :]
        if isinstance(h, int):
            vrows = pl.ds(h * VR, VR)
        else:
            vrows = pl.ds(pl.multiple_of(h * VR, 8), VR)
        ot_s[vrows, col:col + TQ] = o

    def attn_body(hb, carry, last=False):
        if isinstance(hb, int):
            z1 = z2 = 0
        else:
            z1 = jax.lax.shift_right_logical(hb, 16) * CK
            z2 = jax.lax.shift_right_logical(hb, 17) * CK
        deps.clear()
        zv = None if isinstance(hb, int) else jnp.broadcast_to(z1, (8, TQ))
        m8d = {0: carry[0], 1: carry[1]}
        qms = {}
        o = None
        m = None
        for t in range(UPB * NC):
            j, c = divmod(t, NC)
            if c == 0:
                m = jnp.max(m8d[j], axis=0, keepdims=True)
                o = None
            h, col = unit(hb, j)
            o = pv(s_refs[j % 2], h, m, c, o, z2, zv)
            if c == NC - 1:
                finish(h, col, o)
            jq, cq = divmod(t + LAG, NC)
            if last and jq >= UPB:
                if t + LAG == UPB * NC:
                    stage_a2(0, stage_a1(0))
                continue
            if jq not in qms:
                qms[jq] = make_qm(*unit(hb, jq))
            g, qm = qms[jq]
            m8d[jq] = qk(s_refs[jq % 2], g, qm, cq, m8d.get(jq), z1)
        if last:
            return None
        return (m8d[UPB], m8d[UPB + 1])

    cp_wm1.wait()
    cf = c_s[...].astype(F32)
    sc8 = jnp.broadcast_to((cf * jax.nn.sigmoid(cf)).astype(BF16), (8, D))
    mod_s[:, 2 * D:6 * D] = jnp.dot(sc8, wmod_s[:, 2 * D:6 * D], preferred_element_type=F32)
    cp_wo.wait()
    cp_wg.wait()
    cp_wu.wait()
    cp_wd.wait()
    wr_s[0:FR, :] = wgt_s[FM:F, :]
    wr_s[FR:2 * FR, :] = wut_s[FM:F, :]
    wdr_s[0:FR, :] = wd_s[FM:F, :]
    wdr_s[FR:2 * FR, :] = jnp.zeros((FR, D), BF16)
    m8s = {}
    m8 = None
    for t in range(LAG):
        j, c = divmod(t, NC)
        if c == 0:
            g, qm = make_qm(*unit(0, j))
            m8 = None
        m8 = qk(s_refs[j % 2], g, qm, c, m8, 0)
        m8s[j] = m8
    carry = jax.lax.fori_loop(0, H - 1, attn_body, (m8s[0], m8s[1]))
    attn_body(H - 1, carry, last=True)

    def out_copy(i, slot):
        return pltpu.make_async_copy(out_s.at[slot], out_hbm.at[_blk(i), :], out_sems.at[slot])

    def ffn_body(i, carry, last=False):
        slot = i % 2
        gb = mod_s[0:1, 5 * D:6 * D]

        def gu(lo, hi):
            h2 = h2_s[slot]
            gate = jax.lax.dot_general(h2, wgt_s[lo:hi, :], NT, preferred_element_type=F32)
            up = jax.lax.dot_general(h2, wut_s[lo:hi, :], NT, preferred_element_type=F32)
            return (jax.nn.gelu(gate, approximate=True) * up).astype(BF16)

        def gu_rem():
            h2 = h2_s[slot]
            rem = jax.lax.dot_general(h2, wr_s[...], NT, preferred_element_type=F32)
            return (jax.nn.gelu(rem, approximate=True) * pltpu.roll(rem, FR, axis=1)).astype(BF16)

        y = None
        prev = None
        for ci in range(len(FCH) + 1):
            cur = None
            if ci < len(FCH):
                lo, hi = FCH[ci]
                cur = (gu(lo, hi), wd_s, lo, hi) if hi <= FM else (gu_rem(), wdr_s, 0, 2 * FR)
            if ci == A1_AT and not last:
                attn = stage_a1(i + 1)
            if ci == A2_AT and not last:
                stage_a2(i + 1, attn)
            if prev is not None:
                a, w_ref, lo, hi = prev
                yc = jnp.dot(a, w_ref[lo:hi, :], preferred_element_type=F32)
                y = yc if y is None else y + yc
            prev = cur
        res = (x1_s[slot] + gb * y).astype(BF16)

        if last:
            out_copy(i - 2, slot).wait()
        else:
            @pl.when(i >= 2)
            def _():
                out_copy(i - 2, slot).wait()

        out_s[slot] = res
        out_copy(i, slot).start()
        return carry

    jax.lax.fori_loop(0, NBLK - 1, ffn_body, 0)
    ffn_body(NBLK - 1, 0, last=True)
    out_copy(NBLK - 2, (NBLK - 2) % 2).wait()
    out_copy(NBLK - 1, (NBLK - 1) % 2).wait()


@jax.jit
def pallas_adaLN_cond__mha_block__geglu_ffn__prompt_kernel(
    A_x: jax.Array,
    A_wqkv: jax.Array,
    A_wo: jax.Array,
    B_x: jax.Array,
    B_w_gate: jax.Array,
    B_w_up: jax.Array,
    B_w_down: jax.Array,
    c: jax.Array,
    w_mod: jax.Array,
):
    del B_x
    x = A_x.reshape(S, D)
    hbm = pl.BlockSpec(memory_space=pltpu.MemorySpace.HBM)
    scratch = [
        pltpu.VMEM((S, D), BF16),
        pltpu.VMEM((D, 3 * D), BF16),
        pltpu.VMEM((D, D), BF16),
        pltpu.VMEM((F, D), BF16),
        pltpu.VMEM((F, D), BF16),
        pltpu.VMEM((F, D), BF16),
        pltpu.VMEM((1, D), BF16),
        pltpu.VMEM((D, 6 * D), BF16),
        pltpu.VMEM((S, D), BF16),
        pltpu.VMEM((G, S, 128), BF16),
        pltpu.VMEM((G, 128, S), BF16),
        pltpu.VMEM((PADW, S), F32),
        pltpu.VMEM((S, TQ), F32),
        pltpu.VMEM((S, TQ), F32),
        pltpu.VMEM((PADW, S), F32),
        pltpu.VMEM((2 * D, D), BF16),
        pltpu.VMEM((2 * FR, D), BF16),
        pltpu.VMEM((2 * FR, D), BF16),
        pltpu.VMEM((8, 6 * D), F32),
        pltpu.VMEM((2, TB, D), F32),
        pltpu.VMEM((2, TB, D), BF16),
        pltpu.VMEM((2, TB, D), BF16),
        pltpu.SemaphoreType.DMA((10,)),
        pltpu.SemaphoreType.DMA((NBLK,)),
        pltpu.SemaphoreType.DMA((2,)),
    ]
    out = pl.pallas_call(
        _kernel,
        out_shape=jax.ShapeDtypeStruct((S, D), BF16),
        in_specs=[hbm] * 8,
        out_specs=hbm,
        scratch_shapes=scratch,
        compiler_params=pltpu.CompilerParams(vmem_limit_bytes=100 * 1024 * 1024),
    )(x, A_wqkv, A_wo, B_w_gate.T, B_w_up.T, B_w_down, c, w_mod)
    return out.reshape(1, S, D)
```
